```python
import os as _os
_os.environ.setdefault("JAX_PLATFORMS", "cpu")
import jax
import jax.numpy as jnp

def _softmax(x, axis=-1):
    return jax.nn.softmax(x, axis=axis)
def _gelu(x):
    return jax.nn.gelu(x, approximate=True)
def _silu(x):
    return jax.nn.silu(x)
def _sigmoid(x):
    return jax.nn.sigmoid(x)
def _layernorm(x, axis=-1, eps=1e-5):
    m = jnp.mean(x, axis=axis, keepdims=True)
    v = jnp.var(x, axis=axis, keepdims=True)
    return (x - m) / jnp.sqrt(v + eps)
def _scatter_add(tgt, idx, src, axis=0):
    return tgt.at[idx].add(src)
def _segment_sum(src, seg, n):
    return jax.ops.segment_sum(src, seg, n)
class _Rng:
    def __init__(self, key):
        self._k = key
    def _next(self):
        self._k, sub = jax.random.split(self._k)
        return sub
    def normal(self, shape):
        return jax.random.normal(self._next(), shape, dtype=jnp.bfloat16)
    def randint(self, lo, hi, shape):
        return jax.random.randint(self._next(), shape, lo, hi, dtype=jnp.int32)
    def uniform(self, shape, lo=0.0, hi=1.0):
        return jax.random.uniform(self._next(), shape, jnp.bfloat16, lo, hi)
    def permutation(self, n):
        return jax.random.permutation(self._next(), n)


kernel_name = 'concat_heads__mha_block__linear_attn_block__prompt'

def setup_inputs():
    _rng = _Rng(jax.random.key(int.from_bytes(__import__("os").urandom(4), "little")))
    _w = (lambda a: (lambda t: t.astype(jnp.bfloat16) if jnp.issubdtype(t.dtype, jnp.floating) else t)(jnp.asarray(a)))
    def _A_setup():
        B, S, D, H = 1, 2048, 1024, 32
        return {
            "x": _w((lambda *s: _rng.normal(s) * 0.2)(B, S, D)),
            "wqkv": _w((lambda *s: _rng.normal(s) * 0.2)(D, 3 * D)),
            "wo": _w((lambda *s: _rng.normal(s) * 0.05)(D, D)),
        }
    _A_in = _A_setup()

    def _B_setup():
        B, S, D = 1, 2048, 1024
        return {
            "x": _w((lambda *s: _rng.normal(s) * 0.05)(B, S, D)),
            "wqkv": _w((lambda *s: _rng.normal(s) * 1.6)(D, 3 * D)),
            "wo": _w((lambda *s: _rng.normal(s) * 0.1)(D, D)),
        }
    _B_in = _B_setup()

    return {
        "A_x": _A_in["x"],
        "A_wqkv": _A_in["wqkv"],
        "A_wo": _A_in["wo"],
        "B_x": _B_in["x"],
        "B_wqkv": _B_in["wqkv"],
        "B_wo": _B_in["wo"],
    }

def reference(A_x, A_wqkv, A_wo, B_x, B_wqkv, B_wo):
    def _A_ref(x, wqkv, wo):
        B, S, D = x.shape
        H = 32
        Dh = D // H
        qkv = (lambda x, *d: x.transpose(*d))((x @ wqkv).reshape(B, S, 3, H, Dh), 2, 0, 3, 1, 4)
        q, k, v = qkv[0], qkv[1], qkv[2]
        scores = jnp.einsum("bhqd,bhkd->bhqk", q, k) * (Dh ** -0.5)
        p = _softmax(scores, axis=-1)
        o = jnp.einsum("bhqk,bhkd->bhqd", p, v)
        return (lambda x, *d: x.transpose(*d))(o, 0, 2, 1, 3).reshape(B, S, D) @ wo

    def _B_ref(x, wqkv, wo):
        B, S, D = x.shape
        H = 32; Dh = D // H
        qkv = (lambda x, *d: x.transpose(*d))((x @ wqkv).reshape(B, S, 3, H, Dh), 2, 0, 3, 1, 4)
        q, k, v = qkv[0], qkv[1], qkv[2]
        phi = lambda t: jnp.where(t > 0, t + 1, jnp.exp(t)) + 1e-6
        pq, pk = phi(q), phi(k)
        kv = jnp.einsum("bhsd,bhse->bhde", pk, v)
        z = jnp.einsum("bhsd->bhd", pk)
        num = jnp.einsum("bhqd,bhde->bhqe", pq, kv)
        den = jnp.einsum("bhqd,bhd->bhq", pq, z)[..., None] + 1e-6
        o = num / den
        return (lambda x, *d: x.transpose(*d))(o, 0, 2, 1, 3).reshape(B, S, D) @ wo

    a = _A_ref(A_x, A_wqkv, A_wo)
    b = _B_ref(B_x, B_wqkv, B_wo)
    return jnp.concatenate([a, b], axis=-1)
```

```python
import functools
import jax
import jax.numpy as jnp
from jax.experimental import pallas as pl
from jax.experimental.pallas import tpu as pltpu

S = 2048
D = 1024
H = 32
DH = 32
G = D // 128
TM = 512
TQ = 512
TK = 128
LOG2E = 1.4426950408889634
F32 = jnp.float32
BF16 = jnp.bfloat16
NT = (((1,), (1,)), ((), ()))
TN = (((0,), (0,)), ((), ()))


def _dot(a, b):
    return jnp.dot(a, b, preferred_element_type=F32)


def _kernel(xa_hbm, wa_hbm, woa_hbm, xb_hbm, wb_hbm, wob_hbm, out_hbm,
            xa, wa, woa, xb, wb, wob,
            q_s, k_s, vt_s, ot_s, s0, s1, m0, m1, kvw_s, zb_s, out_s,
            sem_in, sem_out):
    nm = S // TM

    def in_copy(src, dst, i):
        return pltpu.make_async_copy(src, dst, sem_in.at[i])

    cps = []
    cps.append(in_copy(xa_hbm.at[0, pl.ds(0, TM)], xa.at[pl.ds(0, TM)], 0))
    for c in range(3):
        cps.append(in_copy(wa_hbm.at[:, pl.ds(c * D, D)], wa.at[c], 1 + c))
    cps.append(in_copy(xa_hbm.at[0, pl.ds(TM, S - TM)], xa.at[pl.ds(TM, S - TM)], 4))
    cps.append(in_copy(woa_hbm, woa, 5))
    cps.append(in_copy(xb_hbm.at[0], xb, 6))
    for c in range(3):
        cps.append(in_copy(wb_hbm.at[:, pl.ds(c * D, D)], wb.at[c], 7 + c))
    cps.append(in_copy(wob_hbm, wob, 10))
    for c in cps:
        c.start()

    cq = float(DH ** -0.5 * LOG2E)
    cps[0].wait()
    cps[1].wait()

    def proj_q(i, _):
        r = pl.ds(pl.multiple_of(i * TM, TM), TM)
        q = _dot(xa[r, :], wa[0]) * cq
        for g in range(G):
            q_s[g, r, :] = q[:, g * 128:(g + 1) * 128].astype(BF16)
        return _
    proj_q(0, 0)
    cps[2].wait()

    def proj_k(i, _):
        r = pl.ds(pl.multiple_of(i * TM, TM), TM)
        k = _dot(xa[r, :], wa[1])
        for g in range(G):
            k_s[g, r, :] = k[:, g * 128:(g + 1) * 128].astype(BF16)
        return _
    proj_k(0, 0)
    cps[4].wait()
    if True:
        jax.lax.fori_loop(1, nm, proj_q, 0)
        jax.lax.fori_loop(1, nm, proj_k, 0)
    cps[3].wait()
    for c in range(D // 256):
        wvt = wa[2, :, c * 256:(c + 1) * 256].T
        for i in range(nm):
            vt_s[c * 256:(c + 1) * 256, i * TM:(i + 1) * TM] = jax.lax.dot_general(
                wvt, xa[i * TM:(i + 1) * TM, :], NT, preferred_element_type=F32).astype(BF16)

    nqb = S // TQ
    nu = H * nqb
    nc = S // TK
    lane = jax.lax.broadcasted_iota(jnp.int32, (TQ // 2, 128), 1)

    def unit(u):
        h = u >> 2
        qb = u & 3
        return h, qb

    def step(u_qk, s_qk, m_qk, u_pv, s_pv, m_pv):
        if u_qk is not None:
            h, qb = unit(u_qk)
            g = h >> 2
            j = h & 3
            qrows = pl.ds(pl.multiple_of(qb * TQ, TQ), TQ)
            qi = pltpu.bitcast(q_s[g, qrows, :], jnp.int32)
            qm = pltpu.bitcast(jnp.where((lane >> 5) == j, qi, 0), BF16)
            mx = None
        if u_pv is not None:
            h2, qb2 = unit(u_pv)
            m = m_pv[...]
            hrows = pl.ds(pl.multiple_of(h2 * DH, DH), DH)
            acc = None
            l = None
        for c in range(nc):
            ks = slice(c * TK, (c + 1) * TK)
            if u_pv is not None:
                s = s_pv[ks, :].reshape(TK // 8, 8, TQ)
                p = jnp.exp2(s - m[None])
                lc = jnp.sum(p, axis=0)
                l = lc if l is None else l + lc
                a = _dot(vt_s[hrows, ks], p.reshape(TK, TQ).astype(BF16))
                acc = a if acc is None else acc + a
            if u_qk is not None:
                s = jax.lax.dot_general(k_s[g, ks, :], qm, NT, preferred_element_type=F32)
                s_qk[ks, :] = s
                mc = jnp.max(s.reshape(TK // 8, 8, TQ), axis=0)
                mx = mc if mx is None else jnp.maximum(mx, mc)
        if u_qk is not None:
            m_qk[...] = jnp.broadcast_to(jnp.max(mx, axis=0, keepdims=True), (8, TQ))
        if u_pv is not None:
            l = jnp.sum(l, axis=0, keepdims=True)
            ot_s[qb2, hrows, :] = (acc / l).astype(BF16)

    step(0, s0, m0, None, None, None)
    step(1, s1, m1, None, None, None)

    def att(i, _):
        u = 2 * i
        step(u + 2, s0, m0, u, s0, m0)
        step(u + 3, s1, m1, u + 1, s1, m1)
        return _
    if True:
        jax.lax.fori_loop(0, nu // 2 - 1, att, 0)
    if True:
        step(None, None, None, nu - 2, s0, m0)
        step(None, None, None, nu - 1, s1, m1)

    cps[5].wait()
    outcps = []
    for i in range(nqb):
        out_s[0, i * TQ:(i + 1) * TQ, :] = jax.lax.dot_general(
            ot_s[i], woa[...], TN, preferred_element_type=F32).astype(BF16)
        cp = pltpu.make_async_copy(out_s.at[0, pl.ds(i * TQ, TQ)],
                                   out_hbm.at[0, pl.ds(i * TQ, TQ), pl.ds(0, D)], sem_out.at[i])
        cp.start()
        outcps.append(cp)

    for c in cps[6:]:
        c.wait()

    def phi(t):
        return jnp.where(t > 0, t + 1.0, jnp.exp(t)) + 1e-6

    def proj_b(i, carry):
        kv, z = carry
        r = pl.ds(pl.multiple_of(i * TM, TM), TM)
        x = xb[r, :]
        pq = phi(_dot(x, wb[0])).astype(BF16)
        for g in range(G):
            q_s[g, r, :] = pq[:, g * 128:(g + 1) * 128]
        pk = phi(_dot(x, wb[1]))
        z = z + jnp.sum(pk.reshape(TM // 8, 8, D), axis=0)
        pk = pk.astype(BF16)
        v = _dot(x, wb[2]).astype(BF16)
        kv = tuple(kv[g] + jax.lax.dot_general(pk[:, g * 128:(g + 1) * 128], v[:, g * 128:(g + 1) * 128], TN,
                                               preferred_element_type=F32) for g in range(G))
        return kv, z
    kv0 = tuple(jnp.zeros((128, 128), F32) for _ in range(G))
    if True:
        kv, z = jax.lax.fori_loop(0, nm, proj_b, (kv0, jnp.zeros((8, D), F32)))
    z = jnp.sum(z, axis=0, keepdims=True)
    ri = jax.lax.broadcasted_iota(jnp.int32, (128, 128), 0) // DH
    ci = jax.lax.broadcasted_iota(jnp.int32, (128, 128), 1) // DH
    bd = ri == ci
    for g in range(G):
        kvg = jnp.where(bd, kv[g], 0.0).astype(BF16)
        kvw_s[g * 128:(g + 1) * 128, :] = _dot(kvg, wob[g * 128:(g + 1) * 128, :]).astype(BF16)
        zg = jnp.broadcast_to(z[:, g * 128:(g + 1) * 128], (128, 128)).T
        zb_s[g] = jnp.where(bd, zg, 0.0).astype(BF16)

    for i in range(nm):
        r = pl.ds(i * TM, TM)
        parts = []
        for g in range(G):
            pq = q_s[g, r, :]
            den = _dot(pq, zb_s[g]) + 1e-6
            parts.append((pq.astype(F32) / den).astype(BF16))
        pqn = jnp.concatenate(parts, axis=1)
        out_s[1, r, :] = _dot(pqn, kvw_s[...]).astype(BF16)
        cp = pltpu.make_async_copy(out_s.at[1, r], out_hbm.at[0, r, pl.ds(D, D)], sem_out.at[nqb + i])
        cp.start()
        outcps.append(cp)
    for cp in outcps:
        cp.wait()


@jax.jit
def pallas_concat_heads__mha_block__linear_attn_block__prompt_kernel(A_x, A_wqkv, A_wo, B_x, B_wqkv, B_wo):
    any_spec = pl.BlockSpec(memory_space=pl.ANY)
    return pl.pallas_call(
        _kernel,
        out_shape=jax.ShapeDtypeStruct((1, S, 2 * D), BF16),
        in_specs=[any_spec] * 6,
        out_specs=any_spec,
        scratch_shapes=[
            pltpu.VMEM((S, D), BF16), pltpu.VMEM((3, D, D), BF16), pltpu.VMEM((D, D), BF16),
            pltpu.VMEM((S, D), BF16), pltpu.VMEM((3, D, D), BF16), pltpu.VMEM((D, D), BF16),
            pltpu.VMEM((G, S, 128), BF16), pltpu.VMEM((G, S, 128), BF16), pltpu.VMEM((D, S), BF16),
            pltpu.VMEM((S // TQ, D, TQ), BF16),
            pltpu.VMEM((S, TQ), F32), pltpu.VMEM((S, TQ), F32), pltpu.VMEM((8, TQ), F32), pltpu.VMEM((8, TQ), F32),
            pltpu.VMEM((D, D), BF16), pltpu.VMEM((G, 128, 128), BF16),
            pltpu.VMEM((2, S, D), BF16),
            pltpu.SemaphoreType.DMA((11,)), pltpu.SemaphoreType.DMA((S // TQ + S // TM,)),
        ],
        compiler_params=pltpu.CompilerParams(vmem_limit_bytes=110 * 1024 * 1024),
        name="fused_mha_linattn",
    )(A_x, A_wqkv, A_wo, B_x, B_wqkv, B_wo)
```

```python
import jax
import jax.numpy as jnp
from jax.experimental import pallas as pl
from jax.experimental.pallas import tpu as pltpu

S = 2048
D = 1024
H = 32
DH = D // H
G = D // 128
TM = 512
TQ = 512
TK = 128
NB = 8
KB = (0, 128, 256, 512, 1024)
TAIL = 2
LOG2E = 1.4426950408889634
F32 = jnp.float32
BF16 = jnp.bfloat16
I32 = jnp.int32
NN = (((1,), (0,)), ((), ()))
NT = (((1,), (1,)), ((), ()))
TN = (((0,), (0,)), ((), ()))
TT = (((0,), (1,)), ((), ()))


def _dot(a, b, dims=NN):
    return jax.lax.dot_general(a, b, dims, preferred_element_type=F32)


def _ds(i, n):
    return pl.ds(i * n if isinstance(i, int) else pl.multiple_of(i * n, n), n)


def _phi(t):
    return jnp.where(t > 0, t + 1.0, jnp.exp(t)) + 1e-6


def _after(x, dep, zero):
    bits = pltpu.bitcast(dep, I32)
    t = zero
    for r in range(dep.shape[0] // 8):
        for c in range(dep.shape[1] // 128):
            t = t & bits[r * 8:(r + 1) * 8, c * 128:(c + 1) * 128]
    xi = pltpu.bitcast(x, I32)
    return pltpu.bitcast(jnp.concatenate([xi[:8] | t, xi[8:]], axis=0), x.dtype)


def _kernel(xa_hbm, wa_hbm, woa_hbm, xb_hbm, wb_hbm, wob_hbm, out_hbm,
            xa, wa, woa, xb, wb, wob,
            q_s, k_s, vt_s, ot_s, s_s, m_s, kvw_s, z_s, out_s, pk_s,
            sem_in, sem_out):
    nm = S // TM
    m0 = 2 * TM
    loads = {}
    stores = []

    def load(name, src, dst):
        loads[name] = pltpu.make_async_copy(src, dst, sem_in.at[len(loads)])
        loads[name].start()

    def wait(*names):
        for name in names:
            loads[name].wait()

    def store(half, rows):
        cp = pltpu.make_async_copy(out_s.at[half, rows], out_hbm.at[0, rows, pl.ds(half * D, D)],
                                   sem_out.at[len(stores)])
        cp.start()
        stores.append(cp)

    for p in range(len(KB) - 1):
        piece = pl.ds(KB[p], KB[p + 1] - KB[p])
        load(f"xa{p}", xa_hbm.at[0, pl.ds(0, m0), piece], xa.at[pl.ds(0, m0), piece])
        load(f"wq{p}", wa_hbm.at[piece, pl.ds(0, D)], wa.at[0, piece])
    load("xa_rest", xa_hbm.at[0, pl.ds(m0, S - m0)], xa.at[pl.ds(m0, S - m0)])
    load("wk", wa_hbm.at[:, pl.ds(D, D)], wa.at[1])
    load("wv", wa_hbm.at[:, pl.ds(2 * D, D)], wa.at[2])
    load("wbk", wb_hbm.at[:, pl.ds(D, D)], wb.at[1])
    load("wbq", wb_hbm.at[:, pl.ds(0, D)], wb.at[0])
    load("wbv", wb_hbm.at[:, pl.ds(2 * D, D)], wb.at[2])
    load("xb", xb_hbm.at[0], xb)
    load("woa", woa_hbm, woa)
    load("wob", wob_hbm, wob)

    qscale = float(DH ** -0.5 * LOG2E)

    def put(dst, rows, y):
        for g in range(G):
            dst[g, rows, :] = y[:, g * 128:(g + 1) * 128].astype(BF16)

    y = None
    for p in range(len(KB) - 1):
        wait(f"xa{p}", f"wq{p}")
        yp = _dot(xa[0:m0, KB[p]:KB[p + 1]], wa[0, KB[p]:KB[p + 1], :])
        y = yp if y is None else y + yp
    put(q_s, pl.ds(0, m0), y * qscale)
    wait("xa_rest")
    for i in range(m0 // TM, nm):
        put(q_s, _ds(i, TM), _dot(xa[_ds(i, TM), :], wa[0]) * qscale)
    wait("wk", "wv", "wbk")
    for i in range(nm):
        put(k_s, _ds(i, TM), _dot(xa[_ds(i, TM), :], wa[1]))
    for c in range(D // 256):
        wvt = wa[2, :, _ds(c, 256)].T
        for i in range(nm):
            vt_s[_ds(c, 256), _ds(i, TM)] = _dot(wvt, xa[_ds(i, TM), :], NT).astype(BF16)

    nqb = S // TQ
    lq = nqb.bit_length() - 1
    nu = H * nqb
    lane_head = jax.lax.broadcasted_iota(I32, (TQ // 2, 128), 1) // DH

    def step(u_qk, u_pv, t, extra=None, zero=None):
        s_ref, m_ref = s_s.at[t], m_s.at[t]
        mx = acc = l = None
        if u_qk is not None:
            h = u_qk >> lq
            g = h >> 2
            q = pltpu.bitcast(q_s[g, _ds(u_qk & (nqb - 1), TQ), :], I32)
            q = pltpu.bitcast(jnp.where(lane_head == (h & 3), q, 0), BF16)
        if u_pv is not None:
            head_rows = _ds(u_pv >> lq, DH)
            m = m_ref[...]
        for c in range(S // TK):
            keys = _ds(c, TK)
            prev = None if acc is None else jnp.concatenate([acc, l], axis=0)
            if u_pv is not None:
                p = jnp.exp2(s_ref[keys, :].reshape(TK // 8, 8, TQ) - m[None])
                lc = jnp.sum(p, axis=0)
                l = lc if l is None else l + lc
                a = _dot(vt_s[head_rows, keys], p.reshape(TK, TQ).astype(BF16))
                acc = a if acc is None else acc + a
            if u_qk is not None:
                k = k_s[g, keys, :]
                if prev is not None:
                    k = _after(k, prev, zero)
                s = _dot(k, q, NT)
                s_ref[keys, :] = s
                mc = jnp.max(s.reshape(TK // 8, 8, TQ), axis=0)
                mx = mc if mx is None else jnp.maximum(mx, mc)
            if extra is not None:
                extra(c)
        if u_qk is not None:
            m_ref[...] = jnp.broadcast_to(jnp.max(mx, axis=0, keepdims=True), (8, TQ))
        if u_pv is not None:
            l = jnp.sum(l, axis=0, keepdims=True)
            ot_s[u_pv & (nqb - 1), head_rows, :] = (acc / l).astype(BF16)

    for t in range(NB):
        step(t, None, t)
        feat = _ds(t, D // NB)
        wa[1, feat, :] = wb[1, :, feat].T

    @pl.loop(0, nu // NB - 1)
    def _(i):
        for t in range(NB):
            step(NB * i + NB + t, NB * i + t, t, zero=i >> 20)

    wait("xb", "wbq", "wbv", "woa", "wob")
    assert NB == G and S // TK == S // 128
    for t in range(NB):
        feat = _ds(t, 128)
        wt = wa[1, feat, :]
        zs = []

        def keys_b(c, feat=feat, wt=wt, zs=zs):
            pk = _phi(_dot(wt, xb[_ds(c, 128), :], NT))
            zs.append(pk if c == 0 else zs[-1] + pk)
            pk_s[c // (TM // 128), feat, _ds(c % (TM // 128), 128)] = pk.astype(BF16)

        step(None, nu - NB + t, t, keys_b)
        z_s[feat, :] = jnp.broadcast_to(jnp.sum(zs[-1], axis=1, keepdims=True), (128, 128))

    for i in range(nqb):
        out_s[0, _ds(i, TQ), :] = _dot(ot_s[i], woa[...], TN).astype(BF16)
        store(0, _ds(i, TQ))

    same_head = (jax.lax.broadcasted_iota(I32, (128, 128), 0) // DH
                 == jax.lax.broadcasted_iota(I32, (128, 128), 1) // DH)
    tf = 256

    def kx(c):
        y = None
        for i in range(nm):
            yi = _dot(pk_s[i, _ds(c, tf), :], xb[_ds(i, TM), :])
            y = yi if y is None else y + yi
        wa[1, _ds(c, tf), :] = y.astype(BF16)

    def kvw(c):
        for g in range(c * tf // 128, (c + 1) * tf // 128):
            grp = _ds(g, 128)
            kv = jnp.where(same_head, _dot(wa[1, grp, :], wb[2, :, grp]), 0.0).astype(BF16)
            kvw_s[grp, :] = _dot(kv, wob[grp, :]).astype(BF16)

    def queries_b(i):
        hd = D // 2
        for c in range(2):
            feat = _ds(c, hd)
            pq = _phi(_dot(wb[0, :, feat], xb[_ds(i, TM), :], TT))
            w = pq * jnp.concatenate([z_s[feat, :]] * (TM // 128), axis=1)
            den = jnp.sum(w.reshape(hd // DH, DH, TM), axis=1, keepdims=True) + 1e-6
            pqn = pq.reshape(hd // DH, DH, TM) * (1.0 / den)
            ot_s[i, feat, :] = pqn.reshape(hd, TM).astype(BF16)

    def out_b(i, parts=1):
        n = TM // parts
        for p in range(parts):
            rows = pl.ds(i * TM + p * n, n)
            out_s[1, rows, :] = _dot(ot_s[i, :, _ds(p, n)], kvw_s[...], TN).astype(BF16)
            store(1, rows)

    for c in range(D // tf):
        kx(c)
        if c > 0:
            kvw(c - 1)
    queries_b(0)
    kvw(D // tf - 1)
    for i in range(1, nm):
        queries_b(i)
        out_b(i - 1)
    out_b(nm - 1, TAIL)
    for cp in stores:
        cp.wait()


@jax.jit
def pallas_concat_heads__mha_block__linear_attn_block__prompt_kernel(
    A_x: jax.Array,
    A_wqkv: jax.Array,
    A_wo: jax.Array,
    B_x: jax.Array,
    B_wqkv: jax.Array,
    B_wo: jax.Array,
):
    any_spec = pl.BlockSpec(memory_space=pl.ANY)
    return pl.pallas_call(
        _kernel,
        out_shape=jax.ShapeDtypeStruct((1, S, 2 * D), BF16),
        in_specs=[any_spec] * 6,
        out_specs=any_spec,
        scratch_shapes=[
            pltpu.VMEM((S, D), BF16), pltpu.VMEM((3, D, D), BF16), pltpu.VMEM((D, D), BF16),
            pltpu.VMEM((S, D), BF16), pltpu.VMEM((3, D, D), BF16), pltpu.VMEM((D, D), BF16),
            pltpu.VMEM((G, S, 128), BF16),
            pltpu.VMEM((G, S, 128), BF16),
            pltpu.VMEM((D, S), BF16),
            pltpu.VMEM((S // TQ, D, TQ), BF16),
            pltpu.VMEM((NB, S, TQ), F32),
            pltpu.VMEM((NB, 8, TQ), F32),
            pltpu.VMEM((D, D), BF16),
            pltpu.VMEM((D, 128), F32),
            pltpu.VMEM((2, S, D), BF16),
            pltpu.VMEM((S // TM, D, TM), BF16),
            pltpu.SemaphoreType.DMA((2 * (len(KB) - 1) + 9,)),
            pltpu.SemaphoreType.DMA((S // TQ + S // TM - 1 + TAIL,)),
        ],
        compiler_params=pltpu.CompilerParams(vmem_limit_bytes=110 * 1024 * 1024),
        name="fused_mha_linattn",
    )(A_x, A_wqkv, A_wo, B_x, B_wqkv, B_wo)
```
